```python
import jax
import jax.numpy as jnp

def _softmax(x, axis=-1):
    return jax.nn.softmax(x, axis=axis)
def _gelu(x):
    return jax.nn.gelu(x, approximate=True)
def _silu(x):
    return jax.nn.silu(x)
def _sigmoid(x):
    return jax.nn.sigmoid(x)
def _layernorm(x, axis=-1, eps=1e-5):
    m = jnp.mean(x, axis=axis, keepdims=True)
    v = jnp.var(x, axis=axis, keepdims=True)
    return (x - m) / jnp.sqrt(v + eps)
def _scatter_add(tgt, idx, src, axis=0):
    return tgt.at[idx].add(src)
def _segment_sum(src, seg, n):
    return jax.ops.segment_sum(src, seg, n)
class _Rng:
    def __init__(self, key):
        self._k = key
    def _next(self):
        self._k, sub = jax.random.split(self._k)
        return sub
    def normal(self, shape):
        return jax.random.normal(self._next(), shape, dtype=jnp.bfloat16)
    def randint(self, lo, hi, shape):
        return jax.random.randint(self._next(), shape, lo, hi, dtype=jnp.int32)
    def uniform(self, shape, lo=0.0, hi=1.0):
        return jax.random.uniform(self._next(), shape, jnp.bfloat16, lo, hi)
    def permutation(self, n):
        return jax.random.permutation(self._next(), n)


kernel_name = 'standalone__batchnorm__prompt'

def setup_inputs():
    _rng = _Rng(jax.random.key(int.from_bytes(__import__("os").urandom(4), "little")))
    _w = (lambda a: (lambda t: t.astype(jnp.bfloat16) if jnp.issubdtype(t.dtype, jnp.floating) else t)(jnp.asarray(a)))
    B, S, C = 2, 2048, 1024
    K = 3
    return {
        "x": _w((lambda *s: _rng.normal(s) * 0.05)(B, S, C)),
        "w": _w((lambda *s: _rng.normal(s) * 0.05)(K, C, C) * (1.0 / (K * C) ** 0.5)),
        "mean": _w((lambda *s: _rng.normal(s) * 0.05)(C) * 0.1),
        "var": _w(jnp.abs((lambda *s: _rng.normal(s) * 0.05)(C)) + 0.5),
        "g": _w((lambda *s: _rng.normal(s) * 0.05)(C) + 1.0),
        "b": _w((lambda *s: _rng.normal(s) * 0.05)(C) * 0.1),
    }

def reference(x, w, mean, var, g, b):
    K = 3
    P = K // 2
    S = x.shape[1]
    xp = jnp.pad(x, ((0, 0), (P, P), (0, 0)))
    y = sum(jnp.einsum('bsc,cd->bsd', xp[:, k:k + S, :], w[k]) for k in range(K))
    inv_std = 1.0 / jnp.sqrt(var + 1e-5)
    y = (y - mean) * (g * inv_std) + b
    return _silu(y)
```

```python
import functools

import jax
import jax.numpy as jnp
from jax import lax
import jax.experimental.pallas as pl
import jax.experimental.pallas.tpu as pltpu

f32 = jnp.float32
bf16 = jnp.bfloat16
i32 = jnp.int32

PA, PB = 2.0 / 3.0, 1.5
PA2, PB2 = PA * PA, PB * PB
NA = 2.0 * PA2 * (PA2 - PB2)
NB = 2.0 * PB2 * (PB2 - PA2)
EPS = 1e-5

TM = 128
TS = 4 * TM
NC = 128
PAD = 16
RI = 32
ORDER = (1, 2, 3, 4, 0, 5)
P1N = 512
DEPTH = 4


def _lo(w):
    return pltpu.bitcast(w << 16, f32)


def _hi(w):
    return pltpu.bitcast(w & -65536, f32)


def _pack(lo_rows, hi_rows):
    return pltpu.pack_elementwise([lo_rows, hi_rows], packed_dtype=bf16)


def _as_bf16(w):
    return pltpu.bitcast(w, bf16)


def _kernel(x_hbm, w_hbm, mean_hbm, var_hbm, g_hbm, b_hbm, o_hbm,
            xbuf, obuf, wbuf, gbuf, u1, ua, ub, acc, mbuf, bn, v0, v1, v2, v3,
            psem, xsem, osem, vsem, *, B, S, C):
    nsl = C // 128
    mpb = S // TS
    nm = B * mpb
    rb = S + PAD
    xi = xbuf.bitcast(i32)
    oi = obuf.bitcast(i32)
    dot = functools.partial(jnp.dot, preferred_element_type=f32)

    def unit_copies(k):
        n0 = 2 * TS + PAD
        cps = [pltpu.make_async_copy(x_hbm.at[0, pl.ds(0, n0), pl.ds(k * 128, 128)],
                                     xbuf.at[k, pl.ds(PAD, n0), :], psem.at[k])]
        cps += [pltpu.make_async_copy(w_hbm.at[t, pl.ds(k * 128, 128), :],
                                      wbuf.at[t, pl.ds(k * 128, 128), :], psem.at[k])
                for t in range(3)]
        return cps

    def x_copies(m):
        bb, j = divmod(m, mpb)
        t0 = j * TS + (PAD if j > 0 else 0)
        t1 = min((j + 1) * TS + PAD, S)
        return [pltpu.make_async_copy(x_hbm.at[bb, pl.ds(t0, t1 - t0), pl.ds(c * 128, 128)],
                                      xbuf.at[c, pl.ds(PAD + bb * rb + t0, t1 - t0), :], xsem.at[m])
                for c in range(nsl)]

    def out_copy(m, n):
        return pltpu.make_async_copy(
            obuf.at[n, pl.ds(m * TS, TS), :],
            o_hbm.at[m // mpb, pl.ds((m % mpb) * TS, TS), pl.ds(n * 128, 128)], osem.at[m])

    vec_copies = [pltpu.make_async_copy(s, d, vsem.at[i]) for i, (s, d) in enumerate(
        ((mean_hbm, v0), (var_hbm, v1), (g_hbm, v2), (b_hbm, v3)))]

    queue = [('u', k) for k in range(nsl)] + [('x', m) for m in range(2, nm)]
    queue.remove(('x', 2))
    queue.insert(nsl - 2, ('x', 2))
    issued = [0]

    def copies_of(item):
        return unit_copies(item[1]) if item[0] == 'u' else x_copies(item[1])

    def issue(count):
        for item in queue[issued[0]:issued[0] + count]:
            for cp in copies_of(item):
                cp.start()
        issued[0] = min(issued[0] + count, len(queue))

    def wait(item):
        assert item in queue[:issued[0]]
        for cp in copies_of(item):
            cp.wait()

    def pin(flag, anchor):
        def f(v):
            return jnp.where(flag, v, pltpu.bitcast(anchor[0:v.shape[0], 0:v.shape[1]], i32))
        return f

    def weight_transform(k, c0, cw, tie):
        rs, cs, hs = pl.ds(k * 128, 128), pl.ds(c0, cw), pl.ds(k * 64, 64)
        w = [pltpu.bitcast(wbuf[t, rs, cs], i32) for t in range(3)]
        if tie is not None:
            w = [tie(v) for v in w]
        halves = []
        for part in (_lo, _hi):
            g0, g1, g2 = part(w[0]), part(w[1]), part(w[2])
            ta = g0 * (1.0 / NA) + g2 * (PA2 / NA)
            sa = g1 * (PA / NA)
            tb = g0 * (1.0 / NB) + g2 * (PB2 / NB)
            sb = g1 * (PB / NB)
            halves.append((ta + sa, ta - sa, tb + sb, tb - sb))
        for j in range(4):
            gbuf[j, hs, cs] = _pack(halves[0][j], halves[1][j])

    def weights(p, k0, kn, cs):
        if p in (0, 5):
            return wbuf[0 if p == 0 else 2, pl.ds(k0, kn), cs]
        return _as_bf16(gbuf[p - 1, pl.ds(k0 // 2, kn // 2), cs])

    def x_base(m, r0):
        v = ((m // mpb) * rb + (m % mpb) * TS) // 2 + 2 * r0
        return v if isinstance(v, int) else pl.multiple_of(v, 8)

    def input_transform(base, c, n, dst, d0, tie):
        xv = xi.at[c, pl.ds(base, 2 * n + PAD), :]
        wd = [xv[pl.ds(7 + j, n // 2, stride=4), :] for j in range(6)]
        e0, e1, e2, e3, e4, e5 = _hi(wd[0]), _lo(wd[1]), _hi(wd[1]), _lo(wd[2]), _hi(wd[2]), _lo(wd[3])
        o2, o3, o4, o5 = _hi(wd[3]), _lo(wd[4]), _hi(wd[4]), _lo(wd[5])

        def bt(d0_, d1, d2, d3, d4, d5):
            al = d4 - PB2 * d2
            be = PA * d3 - (PA * PB2) * d1
            ga = d4 - PA2 * d2
            de = PB * d3 - (PB * PA2) * d1
            return [d0_ - (PA2 + PB2) * d2 + d4, al + be, al - be, ga + de, ga - de,
                    d1 - (PA2 + PB2) * d3 + d5]

        even, odd = bt(e0, e1, e2, e3, e4, e5), bt(e4, e5, o2, o3, o4, o5)
        for p in range(6):
            u = _pack(even[p], odd[p])
            dst[p, pl.ds(d0, n // 2), pl.ds(c * 128, 128)] = u if tie is None else tie(u)

    def epilogue(M, m, n, tie=None):
        ns = pl.ds(n * NC, NC)
        sc, sh = bn[0:1, ns], bn[1:2, ns]
        sa, ta, sb, tb = M[1] + M[2], M[1] - M[2], M[3] + M[4], M[3] - M[4]
        h0 = (M[0] + sa + sb) * sc + sh
        h1 = ta * (PA * sc) + tb * (PB * sc) + sh
        h2 = sa * (PA2 * sc) + sb * (PB2 * sc) + sh
        h3 = (ta * (PA * PA2) + tb * (PB * PB2) + M[5]) * sc + sh
        act = lambda h: h * jnp.tanh(h) + h
        w0, w1 = _pack(act(h0), act(h1)), _pack(act(h2), act(h3))
        if tie is not None:
            w0, w1 = tie(w0), tie(w1)
        ob = m * (TS // 2)
        if not isinstance(ob, int):
            ob = pl.multiple_of(ob, 8)
        ov = oi.at[n, pl.ds(ob, 2 * TM), :]
        ov[pl.ds(0, TM, stride=2), :] = w0
        ov[pl.ds(1, TM, stride=2), :] = w1

    issue(DEPTH)
    for cp in vec_copies:
        cp.start()
    zero = jnp.zeros((PAD, 128), bf16)
    for c in range(nsl):
        for bb in range(B + 1):
            xbuf[c, pl.ds(bb * rb, PAD), :] = zero

    def batchnorm_params():
        for cp in vec_copies:
            cp.wait()
        ld = lambda r: r[...].astype(f32).reshape(1, C)
        scale = ld(v2) * lax.rsqrt(ld(v1) + EPS)
        bn[0:1, :] = scale * 0.5
        bn[1:2, :] = (ld(v3) - ld(v0) * scale) * 0.5

    tm2 = 2 * TM

    def prep_pieces(k):
        wt = [functools.partial(weight_transform, k, cb * 128, 128) for cb in range(nsl)]
        it = [functools.partial(input_transform, x_base(0, r * RI), k, RI, u1, r * RI // 2)
              for r in range(tm2 // RI)]
        out = []
        for i in range(max(len(wt), len(it))):
            out += wt[i:i + 1] + it[i:i + 1]
        return out

    def merge(a_, b_):
        out, ia, ib = [], 0, 0
        while ia < len(a_) or ib < len(b_):
            if ib >= len(b_) or (ia < len(a_) and ia * len(b_) <= ib * len(a_)):
                out.append(a_[ia]); ia += 1
            else:
                out.append(b_[ib]); ib += 1
        return out

    block2 = [functools.partial(input_transform, x_base(2, r * RI), c, RI, ua, r * RI // 2)
              for c in range(nsl) for r in range(TM // RI)]
    block2_steps = (nsl - 4, nsl - 3, nsl - 2)

    wait(('u', 0))
    issue(1)
    for piece in prep_pieces(0):
        piece(None)
    flag0 = jnp.max((xi[0, pl.ds(8, 8), :] & 1) | 1) > 0

    ndot = len(ORDER) * (C // P1N)
    barrier = ndot // 3
    for k in range(nsl - 1):
        pieces = prep_pieces(k + 1)
        if k in block2_steps:
            j, nparts = block2_steps.index(k), len(block2_steps)
            pieces = merge(pieces, block2[j * len(block2) // nparts:(j + 1) * len(block2) // nparts])
        di = 0
        for p in ORDER:
            for h in range(C // P1N):
                cs = pl.ds(h * P1N, P1N)
                mh = dot(_as_bf16(u1[p, :, pl.ds(k * 128, 128)]), weights(p, k * 128, 128, cs))
                acc[p, :, cs] = mh if k == 0 else acc[p, :, cs] + mh
                if di == barrier - 1:
                    wait(('u', k + 1))
                    if k == block2_steps[0]:
                        wait(('x', 2))
                    if k == 2:
                        batchnorm_params()
                    issue(1)
                if di >= barrier:
                    q, nq = di - barrier, ndot - barrier
                    for piece in pieces[q * len(pieces) // nq:(q + 1) * len(pieces) // nq]:
                        piece(pin(flag0, mh))
                di += 1
    k = nsl - 1
    for n in range(nsl):
        ns = pl.ds(n * NC, NC)
        M = [None] * 6
        for p in ORDER:
            M[p] = acc[p, :, ns] + dot(_as_bf16(u1[p, :, pl.ds(k * 128, 128)]), weights(p, k * 128, 128, ns))
        epilogue([v[0:TM] for v in M], 0, n)
        out_copy(0, n).start()
        if n < nsl - 1:
            epilogue([v[TM:tm2] for v in M], 1, n)
            out_copy(1, n).start()
        else:
            for p in range(6):
                mbuf[p] = M[p][TM:tm2]
    issue(len(queue))
    wait(('x', 3))

    npieces = nsl * (TM // RI)

    def row_block(m, ucur, unxt, flag):
        mn = jnp.minimum(m + 1, nm - 1)
        di = 0
        for n in range(nsl):
            ns = pl.ds(n * NC, NC)
            M = [None] * 6
            for p in ORDER:
                M[p] = dot(_as_bf16(ucur[p]), weights(p, 0, C, ns))
                tie = pin(flag, M[p])
                if di == 0:
                    epilogue([mbuf[q] for q in range(6)], m - 1, nsl - 1, tie)
                    out_copy(m - 1, nsl - 1).start()
                lo_ = min(max(di - 1, 0) * npieces // (6 * nsl - 7), npieces)
                hi_ = min(di * npieces // (6 * nsl - 7), npieces)
                for pc in range(lo_, hi_):
                    c, r = divmod(pc, TM // RI)
                    input_transform(x_base(mn, r * RI), c, RI, unxt, r * RI // 2, tie)
                di += 1
            if n < nsl - 1:
                epilogue(M, m, n)
                out_copy(m, n).start()
            else:
                for p in range(6):
                    mbuf[p] = M[p]

    def pair(i, carry):
        for ii in range(1, nm // 2):
            needed = [m for m in (2 * ii + 1, 2 * ii + 2) if 4 <= m < nm]

            @pl.when(i == ii)
            def _():
                for m in needed:
                    wait(('x', m))
        flag = i >= 0
        row_block(2 * i, ua, ub, flag)
        row_block(2 * i + 1, ub, ua, flag)
        return carry

    lax.fori_loop(1, nm // 2, pair, 0)
    epilogue([mbuf[q] for q in range(6)], nm - 1, nsl - 1)
    out_copy(nm - 1, nsl - 1).start()
    for m in range(nm):
        for n in range(nsl):
            out_copy(m, n).wait()


@jax.jit
def pallas_standalone__batchnorm__prompt_kernel(x, w, mean, var, g, b):
    B, S, C = x.shape
    assert w.shape == (3, C, C) and C % 512 == 0 and C // 128 >= 6
    assert S % (2 * TS) == 0 and S // TS >= 4 and (B * S // TS) % 2 == 0
    nsl = C // 128
    nm = B * S // TS
    hbm = pl.BlockSpec(memory_space=pl.ANY)
    return pl.pallas_call(
        functools.partial(_kernel, B=B, S=S, C=C),
        grid=(1,),
        in_specs=[hbm] * 6,
        out_specs=hbm,
        out_shape=jax.ShapeDtypeStruct((B, S, C), x.dtype),
        scratch_shapes=[
            pltpu.VMEM((nsl, PAD + B * (S + PAD), 128), bf16),
            pltpu.VMEM((nsl, B * S, 128), bf16),
            pltpu.VMEM((3, C, C), bf16),
            pltpu.VMEM((4, C // 2, C), i32),
            pltpu.VMEM((6, TM, C), i32),
            pltpu.VMEM((6, TM // 2, C), i32),
            pltpu.VMEM((6, TM // 2, C), i32),
            pltpu.VMEM((6, 2 * TM, C), f32),
            pltpu.VMEM((6, TM, NC), f32),
            pltpu.VMEM((8, C), f32),
        ] + [pltpu.VMEM((C,), bf16)] * 4 + [
            pltpu.SemaphoreType.DMA((nsl,)),
            pltpu.SemaphoreType.DMA((nm,)),
            pltpu.SemaphoreType.DMA((nm,)),
            pltpu.SemaphoreType.DMA((4,)),
        ],
        compiler_params=pltpu.CompilerParams(vmem_limit_bytes=100 * 1024 * 1024),
    )(x, w, mean, var, g, b)
```

```python
import functools

import jax
import jax.numpy as jnp
from jax import lax
import jax.experimental.pallas as pl
import jax.experimental.pallas.tpu as pltpu

f32 = jnp.float32
bf16 = jnp.bfloat16
i32 = jnp.int32

PA, PB = 2.0 / 3.0, 1.5
PA2, PB2 = PA * PA, PB * PB
NA = 2.0 * PA2 * (PA2 - PB2)
NB = 2.0 * PB2 * (PB2 - PA2)
EPS = 1e-5

TM = 128
TS = 4 * TM
NC = 128
PAD = 16
RI = 32
ORDER = (1, 2, 3, 4, 0, 5)
P1N = 512
DEPTH = 4


def _lo(w):
    return pltpu.bitcast(w << 16, f32)


def _hi(w):
    return pltpu.bitcast(w & -65536, f32)


def _pack(lo_rows, hi_rows):
    lo_, hi_ = pltpu.bitcast(lo_rows, i32) + 0x8000, pltpu.bitcast(hi_rows, i32) + 0x8000
    return lax.shift_right_logical(lo_, 16) | (hi_ & -65536)


def _as_bf16(w):
    return pltpu.bitcast(w, bf16)


def _kernel(x_hbm, w_hbm, mean_hbm, var_hbm, g_hbm, b_hbm, o_hbm,
            xbuf, obuf, wbuf, gbuf, u1, ua, ub, acc, mbuf, bn, v0, v1, v2, v3,
            psem, usem, xsem, osem, vsem, *, B, S, C):
    nsl = C // 128
    mpb = S // TS
    nm = B * mpb
    rb = S + PAD
    xi = xbuf.bitcast(i32)
    oi = obuf.bitcast(i32)
    dot = functools.partial(jnp.dot, preferred_element_type=f32)

    def unit_copies(k):
        n0 = 2 * TS + PAD
        sems = [usem.at[j] for j in range(4)] if k == 0 else [psem.at[k]] * 4
        cps = [pltpu.make_async_copy(x_hbm.at[0, pl.ds(0, n0), pl.ds(k * 128, 128)],
                                     xbuf.at[k, pl.ds(PAD, n0), :], sems[0])]
        cps += [pltpu.make_async_copy(w_hbm.at[t, pl.ds(k * 128, 128), :],
                                      wbuf.at[t, pl.ds(k * 128, 128), :], sems[1 + j])
                for j, t in enumerate((0, 2, 1))]
        return cps

    def x_copies(m):
        bb, j = divmod(m, mpb)
        t0 = j * TS + (PAD if j > 0 else 0)
        t1 = min((j + 1) * TS + PAD, S)
        return [pltpu.make_async_copy(x_hbm.at[bb, pl.ds(t0, t1 - t0), pl.ds(c * 128, 128)],
                                      xbuf.at[c, pl.ds(PAD + bb * rb + t0, t1 - t0), :], xsem.at[m])
                for c in range(nsl)]

    def out_copy(m, n):
        return pltpu.make_async_copy(
            obuf.at[n, pl.ds(m * TS, TS), :],
            o_hbm.at[m // mpb, pl.ds((m % mpb) * TS, TS), pl.ds(n * 128, 128)], osem.at[m])

    vec_copies = [pltpu.make_async_copy(s, d, vsem.at[i]) for i, (s, d) in enumerate(
        ((mean_hbm, v0), (var_hbm, v1), (g_hbm, v2), (b_hbm, v3)))]

    queue = [('u', k) for k in range(nsl)] + [('x', m) for m in range(2, nm)]
    queue.remove(('x', 2))
    queue.insert(nsl - 3, ('x', 2))
    issued = [0]

    def copies_of(item):
        return unit_copies(item[1]) if item[0] == 'u' else x_copies(item[1])

    def issue(count):
        for item in queue[issued[0]:issued[0] + count]:
            for cp in copies_of(item):
                cp.start()
        issued[0] = min(issued[0] + count, len(queue))

    def wait(item):
        assert item in queue[:issued[0]]
        for cp in copies_of(item):
            cp.wait()

    def pin(flag, anchor):
        def f(v):
            return jnp.where(flag, v, pltpu.bitcast(anchor[0:v.shape[0], 0:v.shape[1]], i32))
        return f

    def weight_transform(k, c0, cw, tie):
        rs, cs, hs = pl.ds(k * 128, 128), pl.ds(c0, cw), pl.ds(k * 64, 64)
        w = [pltpu.bitcast(wbuf[t, rs, cs], i32) for t in range(3)]
        if tie is not None:
            w[1] = tie(w[1])
        halves = []
        for part in (_lo, _hi):
            g0, g1, g2 = part(w[0]), part(w[1]), part(w[2])
            ta = g0 * (1.0 / NA) + g2 * (PA2 / NA)
            sa = g1 * (PA / NA)
            tb = g0 * (1.0 / NB) + g2 * (PB2 / NB)
            sb = g1 * (PB / NB)
            halves.append((ta + sa, ta - sa, tb + sb, tb - sb))
        for j in range(4):
            gbuf[j, hs, cs] = _pack(halves[0][j], halves[1][j])

    def weights(p, k0, kn, cs):
        if p in (0, 5):
            return wbuf[0 if p == 0 else 2, pl.ds(k0, kn), cs]
        return _as_bf16(gbuf[p - 1, pl.ds(k0 // 2, kn // 2), cs])

    def x_base(m, r0):
        v = ((m // mpb) * rb + (m % mpb) * TS) // 2 + 2 * r0
        return v if isinstance(v, int) else pl.multiple_of(v, 8)

    def input_transform(base, c, n, dst, d0, tie):
        xv = xi.at[c, pl.ds(base, 2 * n + PAD), :]
        wd = [xv[pl.ds(7 + j, n // 2, stride=4), :] for j in range(6)]
        e0, e1, e2, e3, e4, e5 = _hi(wd[0]), _lo(wd[1]), _hi(wd[1]), _lo(wd[2]), _hi(wd[2]), _lo(wd[3])
        o2, o3, o4, o5 = _hi(wd[3]), _lo(wd[4]), _hi(wd[4]), _lo(wd[5])

        def bt(d0_, d1, d2, d3, d4, d5):
            al = d4 - PB2 * d2
            be = PA * d3 - (PA * PB2) * d1
            ga = d4 - PA2 * d2
            de = PB * d3 - (PB * PA2) * d1
            return [d0_ - (PA2 + PB2) * d2 + d4, al + be, al - be, ga + de, ga - de,
                    d1 - (PA2 + PB2) * d3 + d5]

        even, odd = bt(e0, e1, e2, e3, e4, e5), bt(e4, e5, o2, o3, o4, o5)
        for p in range(6):
            u = _pack(even[p], odd[p])
            dst[p, pl.ds(d0, n // 2), pl.ds(c * 128, 128)] = u if tie is None else tie(u)

    def epilogue(M, m, n, tie=None):
        ns = pl.ds(n * NC, NC)
        sc, sh = bn[0:1, ns], bn[1:2, ns]
        sa, ta, sb, tb = M[1] + M[2], M[1] - M[2], M[3] + M[4], M[3] - M[4]
        h0 = (M[0] + sa + sb) * sc + sh
        h1 = ta * (PA * sc) + tb * (PB * sc) + sh
        h2 = sa * (PA2 * sc) + sb * (PB2 * sc) + sh
        h3 = (ta * (PA * PA2) + tb * (PB * PB2) + M[5]) * sc + sh
        act = lambda h: h * jnp.tanh(h) + h
        w0, w1 = _pack(act(h0), act(h1)), _pack(act(h2), act(h3))
        if tie is not None:
            w0, w1 = tie(w0), tie(w1)
        ob = m * (TS // 2)
        if not isinstance(ob, int):
            ob = pl.multiple_of(ob, 8)
        ov = oi.at[n, pl.ds(ob, 2 * TM), :]
        ov[pl.ds(0, TM, stride=2), :] = w0
        ov[pl.ds(1, TM, stride=2), :] = w1

    issue(DEPTH)
    for cp in vec_copies:
        cp.start()
    zero = jnp.zeros((PAD, 128), bf16)
    for c in range(nsl):
        for bb in range(B + 1):
            xbuf[c, pl.ds(bb * rb, PAD), :] = zero

    def batchnorm_params():
        for cp in vec_copies:
            cp.wait()
        ld = lambda r: r[...].astype(f32).reshape(1, C)
        scale = ld(v2) * lax.rsqrt(ld(v1) + EPS)
        bn[0:1, :] = scale * 0.5
        bn[1:2, :] = (ld(v3) - ld(v0) * scale) * 0.5

    tm2 = 2 * TM

    def prep_pieces(k):
        wt = [functools.partial(weight_transform, k, cb * 128, 128) for cb in range(nsl)]
        it = [functools.partial(input_transform, x_base(0, r * RI), k, RI, u1, r * RI // 2)
              for r in range(tm2 // RI)]
        out = []
        for i in range(max(len(wt), len(it))):
            out += wt[i:i + 1] + it[i:i + 1]
        return out

    def merge(a_, b_):
        out, ia, ib = [], 0, 0
        while ia < len(a_) or ib < len(b_):
            if ib >= len(b_) or (ia < len(a_) and ia * len(b_) <= ib * len(a_)):
                out.append(a_[ia]); ia += 1
            else:
                out.append(b_[ib]); ib += 1
        return out

    block2 = [functools.partial(input_transform, x_base(2, r * RI), c, RI, ua, r * RI // 2)
              for c in range(nsl) for r in range(TM // RI)]
    block2_steps = tuple(range(nsl - 5, nsl - 1))
    waits = {k: [('u', k + 1)] for k in range(nsl - 3)}
    waits[block2_steps[0]].append(('x', 2))
    waits[nsl - 3] = [('u', nsl - 2), ('u', nsl - 1)]
    waits[nsl - 2] = []

    first = unit_copies(0)
    first[0].wait()
    issue(1)
    transform_w0, transform_x0 = prep_pieces(0)[0::2], prep_pieces(0)[1::2]
    for piece in transform_x0:
        piece(None)
    flag0 = jnp.max((xi[0, pl.ds(8, 8), :] & 1) | 1) > 0

    nh = C // P1N
    ndot = len(ORDER) * nh
    for k in range(nsl - 1):
        pieces = prep_pieces(k + 1)
        if k in block2_steps:
            j, nparts = block2_steps.index(k), len(block2_steps)
            pieces = merge(pieces, block2[j * len(block2) // nparts:(j + 1) * len(block2) // nparts])
        order = (0, 5, 1, 2, 3, 4) if k == 0 else ORDER
        barrier = 2 * ndot // 3 if k == 0 else (ndot // 4 if waits[k] else 0)
        di = 0
        for ip, p in enumerate(order):
            if k == 0 and ip < 3:
                first[1 + ip].wait()
                if ip == 2:
                    for piece in transform_w0:
                        piece(None)
            for h in range(nh):
                cs = pl.ds(h * P1N, P1N)
                mh = dot(_as_bf16(u1[p, :, pl.ds(k * 128, 128)]), weights(p, k * 128, 128, cs))
                acc[p, :, cs] = mh if k == 0 else acc[p, :, cs] + mh
                if di == barrier - 1:
                    for item in waits[k]:
                        wait(item)
                    if k == 2:
                        batchnorm_params()
                    issue(1)
                if di >= barrier:
                    q, nq = di - barrier, ndot - barrier
                    for piece in pieces[q * len(pieces) // nq:(q + 1) * len(pieces) // nq]:
                        piece(pin(flag0, mh))
                di += 1
    k = nsl - 1
    for n in range(nsl):
        ns = pl.ds(n * NC, NC)
        M = [None] * 6
        for p in ORDER:
            M[p] = acc[p, :, ns] + dot(_as_bf16(u1[p, :, pl.ds(k * 128, 128)]), weights(p, k * 128, 128, ns))
        epilogue([v[0:TM] for v in M], 0, n)
        out_copy(0, n).start()
        if n < nsl - 1:
            epilogue([v[TM:tm2] for v in M], 1, n)
            out_copy(1, n).start()
        else:
            for p in range(6):
                mbuf[p] = M[p][TM:tm2]
    issue(len(queue))
    wait(('x', 3))

    npieces = nsl * (TM // RI)

    def row_block(m, ucur, unxt, flag):
        mn = jnp.minimum(m + 1, nm - 1)
        di = 0
        for n in range(nsl):
            ns = pl.ds(n * NC, NC)
            M = [None] * 6
            for p in ORDER:
                M[p] = dot(_as_bf16(ucur[p]), weights(p, 0, C, ns))
                tie = pin(flag, M[p])
                if di == 0:
                    epilogue([mbuf[q] for q in range(6)], m - 1, nsl - 1, tie)
                    out_copy(m - 1, nsl - 1).start()
                lo_ = min(max(di - 1, 0) * npieces // (6 * nsl - 7), npieces)
                hi_ = min(di * npieces // (6 * nsl - 7), npieces)
                for pc in range(lo_, hi_):
                    c, r = divmod(pc, TM // RI)
                    input_transform(x_base(mn, r * RI), c, RI, unxt, r * RI // 2, tie)
                di += 1
            if n < nsl - 1:
                epilogue(M, m, n)
                out_copy(m, n).start()
            else:
                for p in range(6):
                    mbuf[p] = M[p]

    def pair(i, carry):
        for ii in range(1, nm // 2):
            needed = [m for m in (2 * ii + 1, 2 * ii + 2) if 4 <= m < nm]

            @pl.when(i == ii)
            def _():
                for m in needed:
                    wait(('x', m))
        flag = i >= 0
        row_block(2 * i, ua, ub, flag)
        row_block(2 * i + 1, ub, ua, flag)
        return carry

    lax.fori_loop(1, nm // 2, pair, 0)
    epilogue([mbuf[q] for q in range(6)], nm - 1, nsl - 1)
    out_copy(nm - 1, nsl - 1).start()
    for m in range(nm):
        for n in range(nsl):
            out_copy(m, n).wait()


@jax.jit
def pallas_standalone__batchnorm__prompt_kernel(x, w, mean, var, g, b):
    B, S, C = x.shape
    assert w.shape == (3, C, C) and C % 512 == 0 and C // 128 >= 6
    assert S % (2 * TS) == 0 and S // TS >= 4 and (B * S // TS) % 2 == 0
    nsl = C // 128
    nm = B * S // TS
    hbm = pl.BlockSpec(memory_space=pl.ANY)
    return pl.pallas_call(
        functools.partial(_kernel, B=B, S=S, C=C),
        grid=(1,),
        in_specs=[hbm] * 6,
        out_specs=hbm,
        out_shape=jax.ShapeDtypeStruct((B, S, C), x.dtype),
        scratch_shapes=[
            pltpu.VMEM((nsl, PAD + B * (S + PAD), 128), bf16),
            pltpu.VMEM((nsl, B * S, 128), bf16),
            pltpu.VMEM((3, C, C), bf16),
            pltpu.VMEM((4, C // 2, C), i32),
            pltpu.VMEM((6, TM, C), i32),
            pltpu.VMEM((6, TM // 2, C), i32),
            pltpu.VMEM((6, TM // 2, C), i32),
            pltpu.VMEM((6, 2 * TM, C), f32),
            pltpu.VMEM((6, TM, NC), f32),
            pltpu.VMEM((8, C), f32),
        ] + [pltpu.VMEM((C,), bf16)] * 4 + [
            pltpu.SemaphoreType.DMA((nsl,)),
            pltpu.SemaphoreType.DMA((4,)),
            pltpu.SemaphoreType.DMA((nm,)),
            pltpu.SemaphoreType.DMA((nm,)),
            pltpu.SemaphoreType.DMA((4,)),
        ],
        compiler_params=pltpu.CompilerParams(vmem_limit_bytes=100 * 1024 * 1024),
    )(x, w, mean, var, g, b)
```
